```python
import jax
import jax.numpy as jnp

def _softmax(x, axis=-1):
    return jax.nn.softmax(x, axis=axis)
def _gelu(x):
    return jax.nn.gelu(x, approximate=True)
def _silu(x):
    return jax.nn.silu(x)
def _sigmoid(x):
    return jax.nn.sigmoid(x)
def _layernorm(x, axis=-1, eps=1e-5):
    m = jnp.mean(x, axis=axis, keepdims=True)
    v = jnp.var(x, axis=axis, keepdims=True)
    return (x - m) / jnp.sqrt(v + eps)
def _scatter_add(tgt, idx, src, axis=0):
    return tgt.at[idx].add(src)
def _segment_sum(src, seg, n):
    return jax.ops.segment_sum(src, seg, n)
class _Rng:
    def __init__(self, key):
        self._k = key
    def _next(self):
        self._k, sub = jax.random.split(self._k)
        return sub
    def normal(self, shape):
        return jax.random.normal(self._next(), shape, dtype=jnp.bfloat16)
    def randint(self, lo, hi, shape):
        return jax.random.randint(self._next(), shape, lo, hi, dtype=jnp.int32)
    def uniform(self, shape, lo=0.0, hi=1.0):
        return jax.random.uniform(self._next(), shape, jnp.bfloat16, lo, hi)
    def permutation(self, n):
        return jax.random.permutation(self._next(), n)


kernel_name = 'recurrent_scan__sliding_block_cached__dense_activation_gelu__decode'

def setup_inputs():
    _rng = _Rng(jax.random.key(int.from_bytes(__import__("os").urandom(4), "little")))
    _w = (lambda a: (lambda t: t.astype(jnp.bfloat16) if jnp.issubdtype(t.dtype, jnp.floating) else t)(jnp.asarray(a)))
    def _A_setup():
        B, Sq, D = 2, 1, 576
        Hq, Hkv, Sk, Dh = 32, 16, 32768, 128
        assert Hq % Hkv == 0, (Hq, Hkv)
        return {
            "x": _w((lambda *s: _rng.normal(s) * 0.05)(B, Sq, D)),
            "k_cache": _w((lambda *s: _rng.normal(s) * 0.05)(B, Hkv, Sk, Dh)),
            "v_cache": _w((lambda *s: _rng.normal(s) * 0.05)(B, Hkv, Sk, Dh)),
            "wq": _w((lambda *s: _rng.normal(s) * 0.05)(D, Hq * Dh) * (D ** -0.5)),
            "wo": _w((lambda *s: _rng.normal(s) * 0.05)(Hq * Dh, D) * ((Hq * Dh) ** -0.5)),
        }
    _A_in = _A_setup()

    def _B_setup():
        B, S, D, F = 2, 1, 576, 4608
        return {
            "x": _w((lambda *s: _rng.normal(s) * 0.05)(B, S, D)),
            "w1": _w((lambda *s: _rng.normal(s) * 0.05)(D, F) * (D ** -0.5)),
            "b1": _w((lambda *s: _rng.normal(s) * 0.05)(F) * 0.01),
            "w2": _w((lambda *s: _rng.normal(s) * 0.05)(F, D) * (F ** -0.5)),
            "b2": _w((lambda *s: _rng.normal(s) * 0.05)(D) * 0.01),
        }
    _B_in = _B_setup()

    return {
        "A_x": _A_in["x"],
        "A_k_cache": _A_in["k_cache"],
        "A_v_cache": _A_in["v_cache"],
        "A_wq": _A_in["wq"],
        "A_wo": _A_in["wo"],
        "B_x": _B_in["x"],
        "B_w1": _B_in["w1"],
        "B_b1": _B_in["b1"],
        "B_w2": _B_in["w2"],
        "B_b2": _B_in["b2"],
    }

def reference(A_x, A_k_cache, A_v_cache, A_wq, A_wo, B_x, B_w1, B_b1, B_w2, B_b2):
    def _A_ref(x, k_cache, v_cache, wq, wo):
        B, Sq, D = x.shape
        Hq, Dh = 32, 128
        Hkv, Sk = k_cache.shape[1], k_cache.shape[2]
        W = min(4096, max(256, Sk // 4))
        rep = Hq // Hkv
        q = (lambda x, *d: x.transpose(*d))((x @ wq).reshape(B, Sq, Hq, Dh), 0, 2, 1, 3)
        k = jnp.repeat(k_cache[:, :, Sk - W:, :], rep, axis=1)
        v = jnp.repeat(v_cache[:, :, Sk - W:, :], rep, axis=1)
        scores = jnp.einsum("bhqd,bhkd->bhqk", q, k) * (Dh ** -0.5)
        p = _softmax(scores, axis=-1)
        o = jnp.einsum("bhqk,bhkd->bhqd", p, v)
        return (lambda x, *d: x.transpose(*d))(o, 0, 2, 1, 3).reshape(B, Sq, Hq * Dh) @ wo

    def _B_ref(x, w1, b1, w2, b2):
        h = jnp.einsum("bsd,df->bsf", x, w1) + b1
        h = _gelu(h)
        return jnp.einsum("bsf,fd->bsd", h, w2) + b2

    x = A_x
    xn = _layernorm(x, axis=-1)
    s = _A_ref(xn, A_k_cache, A_v_cache, A_wq, A_wo)
    g = _silu(_B_ref(xn, B_w1, B_b1, B_w2, B_b2))
    return x + s * g
```

```python
import functools
import jax
import jax.numpy as jnp
from jax import lax
import jax.experimental.pallas as pl
import jax.experimental.pallas.tpu as pltpu

HQ, DH = 32, 128
NT = (((1,), (1,)), ((), ()))
F32, BF16 = jnp.float32, jnp.bfloat16
GH = 4
SR = 256
PR = 128


def make():
  def kernel(x_hbm, k_hbm, v_hbm, wq_hbm, wot_hbm, w1_hbm, b1_hbm, w2t_hbm, b2_hbm,
             o_ref,
             x_v, b1_v, b2_v, wq_v, wo_v, w1_v, w2_v, kbuf, vbuf, q_s, s_s, o_s, h_s,
             sem_s, sem_w, sem_o, sem_2, sem_k, sem_v):
    B, Hkv, Sk, _ = k_hbm.shape
    D = x_hbm.shape[1]
    F = w1_hbm.shape[1]
    A = HQ * DH
    W = kbuf.shape[2]
    NS = W // SR
    NG = Hkv // GH
    LAG = NS // 2

    def mult(i, n):
      return i * n if isinstance(i, int) else pl.multiple_of(i * n, n)

    def issue_kv(src, dst, sem, g, i):
      for j in range(SR // PR):
        r = i * (SR // PR) + j
        n = 0
        for b in range(B):
          for dh in range(GH):
            pltpu.make_async_copy(
                src.at[b, g * GH + dh, pl.ds(Sk - W + mult(r, PR), PR), :],
                dst.at[dh, b, pl.ds(mult(r, PR), PR), :], sem.at[i]).start(priority=n % 2)
            n += 1

    def wait_kv(buf, sem, i):
      view = buf.at[:, :, pl.ds(mult(i, SR), SR), :]
      pltpu.make_async_copy(view, view, sem.at[i]).wait()

    def issue_spread(src, dst, sem, i):
      half = src.shape[1] // 2
      for j in range(2):
        n = 0
        for c in range(2):
          for s in range(4):
            rs = pl.ds(s * (D // 4) + mult(2 * i + j, 8), 8)
            cs = pl.ds(c * half, half)
            pltpu.make_async_copy(src.at[rs, cs], dst.at[rs, cs], sem).start(priority=n % 2)
            n += 1

    def issue_rows(src, dst, sem, i):
      for j in range(2):
        n = 0
        for c in range(2):
          for s in range(4):
            rs = pl.ds(mult(8 * i + 2 * s + j, 8), 8)
            cs = pl.ds(c * (A // 2), A // 2)
            pltpu.make_async_copy(src.at[rs, cs], dst.at[rs, cs], sem.at[i]).start(priority=n % 2)
            n += 1

    def wait_rows(buf, sem, i):
      view = buf.at[pl.ds(64 * i, 64), pl.ds(0, A)]
      pltpu.make_async_copy(view, view, sem.at[i]).wait()

    NSTRIP = (F - A) // 256
    def issue_strip(t):
      n = 0
      for c in range(2):
        for s in range(4):
          rs = pl.ds(s * (D // 4), D // 4)
          cs = pl.ds(A + (2 * t + c) * 128, 128)
          pltpu.make_async_copy(w2t_hbm.at[rs, cs], w2_v.at[rs, cs], sem_2.at[9 + t]).start(priority=n % 2)
          n += 1

    def wait_strip(t):
      view = w2_v.at[:, pl.ds(A + 256 * t, 256)]
      pltpu.make_async_copy(view, view, sem_2.at[9 + t]).wait()

    cp_x = pltpu.make_async_copy(x_hbm, x_v, sem_s.at[0])
    cp_b1 = pltpu.make_async_copy(b1_hbm, b1_v, sem_s.at[1])
    cp_b2 = pltpu.make_async_copy(b2_hbm, b2_v, sem_s.at[2])
    cp_x.start()
    cp_b1.start()
    cp_b2.start()
    lax.fori_loop(0, 9, lambda i, _: issue_spread(wq_hbm, wq_v, sem_w.at[0], i), None)

    cp_x.wait()
    xf = x_v[...].astype(F32)
    mu = jnp.mean(xf, axis=-1, keepdims=True)
    xc = xf - mu
    var = jnp.mean(xc * xc, axis=-1, keepdims=True)
    xn = xc / jnp.sqrt(var + 1e-5)
    row = lax.broadcasted_iota(jnp.int32, (8, D), 0)
    xn8 = jnp.where(row % 2 == 0, xn[0:1, :], xn[1:2, :]).astype(BF16)

    lax.fori_loop(0, 9, lambda i, _: issue_spread(w1_hbm, w1_v, sem_w.at[1], i), None)

    row128 = lax.broadcasted_iota(jnp.int32, (8, DH), 0)
    pltpu.make_async_copy(wq_v, wq_v, sem_w.at[0]).wait()
    for u in range(4):
      issue_kv(k_hbm, kbuf, sem_k, 0, u)
      qq = jnp.dot(xn8, wq_v[:, u * (A // 4):(u + 1) * (A // 4)], preferred_element_type=F32)
      for hh in range(Hkv // 4):
        q_s[u * (Hkv // 4) + hh] = jnp.where(
            row128 < 2, qq[:, 2 * hh * DH:(2 * hh + 1) * DH], qq[:, (2 * hh + 1) * DH:(2 * hh + 2) * DH])
    pltpu.make_async_copy(w1_v, w1_v, sem_w.at[1]).wait()
    cp_b1.wait()
    cp_b2.wait()
    b1 = b1_v[...].astype(F32).reshape(1, F)
    for u in range(4):
      issue_kv(k_hbm, kbuf, sem_k, 0, 4 + u)
      cs = slice(u * (F // 4), (u + 1) * (F // 4))
      hh = jnp.dot(xn8, w1_v[:, cs], preferred_element_type=F32) + b1[:, cs]
      h_s[:, cs] = jax.nn.gelu(hh, approximate=True).astype(BF16)

    scale = DH ** -0.5
    even = lax.broadcasted_iota(jnp.int32, (8, SR), 0) % 2 == 0

    def group(g, _):
      qs = [q_s[g * GH + dh].astype(BF16) for dh in range(GH)]

      def qk(i, ms):
        wait_kv(kbuf, sem_k, i)
        rs = pl.ds(mult(i, SR), SR)
        out = []
        for dh in range(GH):
          s0 = lax.dot_general(qs[dh], kbuf[dh, 0, rs, :], NT, preferred_element_type=F32)
          s1 = lax.dot_general(qs[dh], kbuf[dh, 1, rs, :], NT, preferred_element_type=F32)
          s = jnp.where(even, s0, s1) * scale
          s_s[dh, :, rs] = s
          m = ms[dh]
          for j in range(SR // DH):
            m = jnp.maximum(m, s[:, j * DH:(j + 1) * DH])
          out.append(m)
        return out

      def seg_a(i, ms):
        issue_kv(k_hbm, kbuf, sem_k, g, i + LAG)
        return qk(i, ms)

      def seg_b(i, ms):
        issue_kv(v_hbm, vbuf, sem_v, g, i - LAG)
        return qk(i, ms)

      ms = [jnp.full((8, DH), -jnp.inf, F32)] * GH
      ms = lax.fori_loop(0, LAG, seg_a, ms)
      ms = lax.fori_loop(LAG, NS, seg_b, ms)
      ms = [jnp.max(m, axis=-1, keepdims=True) for m in ms]

      def pv(i, c):
        os_, ls = c
        wait_kv(vbuf, sem_v, i)
        rs = pl.ds(mult(i, SR), SR)
        no, nl = [], []
        for dh in range(GH):
          e = jnp.exp(s_s[dh, :, rs] - ms[dh])
          l = ls[dh]
          for j in range(SR // DH):
            l = l + e[:, j * DH:(j + 1) * DH]
          nl.append(l)
          p = e.astype(BF16)
          for b in range(B):
            no.append(os_[dh * B + b] + jnp.dot(p, vbuf[dh, b, rs, :], preferred_element_type=F32))
        return no, nl

      def seg_c(i, c):
        issue_kv(v_hbm, vbuf, sem_v, g, i + LAG)
        return pv(i, c)

      def seg_d(i, c):
        @pl.when(g + 1 < NG)
        def _():
          issue_kv(k_hbm, kbuf, sem_k, g + 1, i - LAG)
        @pl.when(g + 1 == NG)
        def _():
          issue_rows(wot_hbm, wo_v, sem_o, i - LAG)
        return pv(i, c)

      z = jnp.zeros((8, DH), F32)
      c = ([z] * (GH * B), [z] * GH)
      c = lax.fori_loop(0, LAG, seg_c, c)
      os_, ls = lax.fori_loop(LAG, NS, seg_d, c)
      for dh in range(GH):
        l = jnp.sum(ls[dh], axis=-1, keepdims=True)
        o_s[g * GH + dh] = jnp.where(row128 % 2 == 0, os_[dh * B], os_[dh * B + 1]) / l
      return None

    lax.fori_loop(0, NG, group, None)

    parts = []
    for h in range(Hkv):
      ob = o_s[h]
      parts += [jnp.where(row128 < 2, ob, 0.0), jnp.where(row128 < 2, 0.0, ob)]
    lhs = jnp.concatenate(parts, axis=1).astype(BF16)

    pending = [functools.partial(issue_rows, wot_hbm, wo_v, sem_o, i) for i in range(LAG, 9)]
    pending += [functools.partial(issue_rows, w2t_hbm, w2_v, sem_2, i) for i in range(9)]
    pending += [lambda: [issue_strip(t) for t in range(NSTRIP)]]

    def proj(lhs, w_v, sem):
      outs = []
      for rb in range(pl.cdiv(D, 128)):
        n = min(128, D - rb * 128)
        for i in range(n // 64):
          if pending:
            pending.pop(0)()
        for i in range(n // 64):
          wait_rows(w_v, sem, 2 * rb + i)
        outs.append(lax.dot_general(lhs, w_v[rb * 128:rb * 128 + n, 0:A], NT, preferred_element_type=F32))
      return jnp.concatenate(outs, axis=1)

    acc = proj(lhs, wo_v, sem_o)
    att = acc[0:2] + acc[2:4]
    f = proj(h_s[:, 0:A], w2_v, sem_2)
    assert not pending
    for t in range(NSTRIP):
      wait_strip(t)
      cs = slice(A + 256 * t, A + 256 * (t + 1))
      f += lax.dot_general(h_s[:, cs], w2_v[:, cs], NT, preferred_element_type=F32)
    ff = f[0:2] + b2_v[...].astype(F32).reshape(1, D)
    g = ff * jax.nn.sigmoid(ff)
    o_ref[...] = (xf + att * g).astype(o_ref.dtype)

  @jax.jit
  def run(A_x, A_k_cache, A_v_cache, A_wq, A_wo, B_x, B_w1, B_b1, B_w2, B_b2):
    B, Sq, D = A_x.shape
    F = B_w1.shape[1]
    Hkv, Sk = A_k_cache.shape[1:3]
    W = min(4096, max(256, Sk // 4))
    hbm = pl.BlockSpec(memory_space=pltpu.HBM)
    out = pl.pallas_call(
        kernel,
        out_shape=jax.ShapeDtypeStruct((B, D), A_x.dtype),
        in_specs=[hbm] * 9,
        out_specs=pl.BlockSpec(memory_space=pltpu.VMEM),
        scratch_shapes=[
            pltpu.VMEM((B, D), BF16), pltpu.VMEM((F,), BF16), pltpu.VMEM((D,), BF16),
            pltpu.VMEM((D, HQ * DH), BF16), pltpu.VMEM((D, HQ * DH), BF16),
            pltpu.VMEM((D, F), BF16), pltpu.VMEM((D, F), BF16),
            pltpu.VMEM((GH, B, W, DH), BF16), pltpu.VMEM((GH, B, W, DH), BF16),
            pltpu.VMEM((Hkv, 8, DH), F32), pltpu.VMEM((GH, 8, W), F32), pltpu.VMEM((Hkv, 8, DH), F32),
            pltpu.VMEM((8, F), BF16),
            pltpu.SemaphoreType.DMA((3,)), pltpu.SemaphoreType.DMA((2,)),
            pltpu.SemaphoreType.DMA((9,)), pltpu.SemaphoreType.DMA((9 + (F - HQ * DH) // 256,)),
            pltpu.SemaphoreType.DMA((W // SR,)), pltpu.SemaphoreType.DMA((W // SR,)),
        ],
        compiler_params=pltpu.CompilerParams(vmem_limit_bytes=64 * 1024 * 1024),
    )(A_x.reshape(B, D), A_k_cache, A_v_cache, A_wq, A_wo.T, B_w1, B_b1, B_w2.T, B_b2)
    return out.reshape(B, Sq, D)
  return run


pallas_recurrent_scan__sliding_block_cached__dense_activation_gelu__decode_kernel = make()
```

```python
import functools

import jax
import jax.numpy as jnp
from jax import lax
import jax.experimental.pallas as pl
import jax.experimental.pallas.tpu as pltpu

HQ, DH = 32, 128
NT = (((1,), (1,)), ((), ()))
F32, BF16 = jnp.float32, jnp.bfloat16
GH = 4
SR = 256
PR = 128
WR = 64


def _kernel(x_hbm, k_hbm, v_hbm, wq_hbm, wot_hbm, w1_hbm, b1_hbm, w2t_hbm, b2_hbm,
            o_ref,
            x_v, b1_v, b2_v, wq_v, wo_v, w1_v, w2_v, kbuf, vbuf, q_s, s_s, o_s, h_s,
            sem_s, sem_w, sem_o, sem_2, sem_k, sem_v):
  B, Hkv, Sk, _ = k_hbm.shape
  D = x_hbm.shape[1]
  F = w1_hbm.shape[1]
  A = HQ * DH
  W = kbuf.shape[2]
  NS = W // SR
  NG = Hkv // GH
  NW = D // WR
  LAG = min(6, NS // 2)

  def mult(i, n):
    return i * n if isinstance(i, int) else pl.multiple_of(i * n, n)

  def start_all(copies):
    for n, c in enumerate(copies):
      c.start(priority=n % 2)

  def wait_for(view, sem):
    pltpu.make_async_copy(view, view, sem).wait()

  def issue_kv(src, dst, sem, g, i):
    start_all([
        pltpu.make_async_copy(
            src.at[b, g * GH + dh, pl.ds(Sk - W + mult(i * (SR // PR) + j, PR), PR), :],
            dst.at[dh, b, pl.ds(mult(i * (SR // PR) + j, PR), PR), :], sem.at[i])
        for j in range(SR // PR) for b in range(B) for dh in range(GH)])

  def wait_kv(buf, sem, i):
    wait_for(buf.at[:, :, pl.ds(mult(i, SR), SR), :], sem.at[i])

  def wcopy(src, dst, sem, rs, cs):
    return pltpu.make_async_copy(src.at[rs, cs], dst.at[rs, cs], sem)

  def issue_spread(src, dst, sem, i):
    half = src.shape[1] // 2
    start_all([
        wcopy(src, dst, sem, pl.ds(s * (D // 4) + mult(2 * i + j, 8), 8), pl.ds(c * half, half))
        for j in range(2) for c in range(2) for s in range(4)])

  def issue_wo(i):
    start_all([
        wcopy(wot_hbm, wo_v, sem_o.at[i], pl.ds(mult(8 * i + 2 * s + j, 8), 8),
              pl.ds(c * (A // 2), A // 2))
        for j in range(2) for c in range(2) for s in range(4)])

  def w2_unit(u):
    if u < NW - 1:
      return pl.ds(WR * u, WR), pl.ds(0, F)
    return pl.ds(D - WR, WR), pl.ds((u - NW + 1) * (F // 2), F // 2)

  def issue_w2(i):
    copies = []
    for c in range(2):
      for s in range(4):
        for u in (i // 2 * 2, i // 2 * 2 + 1):
          if u < NW - 1:
            rs, cs = pl.ds(WR * u + 8 * (2 * s + i % 2), 8), pl.ds(c * (F // 2), F // 2)
          else:
            rs, cs = pl.ds(D - WR + 8 * (2 * s + c), 8), w2_unit(u)[1]
          copies.append(wcopy(w2t_hbm, w2_v, sem_2.at[u], rs, cs))
    start_all(copies)

  cp_x = pltpu.make_async_copy(x_hbm, x_v, sem_s.at[0])
  cp_b1 = pltpu.make_async_copy(b1_hbm, b1_v, sem_s.at[1])
  cp_b2 = pltpu.make_async_copy(b2_hbm, b2_v, sem_s.at[2])
  cp_x.start()
  cp_b1.start()
  cp_b2.start()
  lax.fori_loop(0, NW, lambda i, _: issue_spread(wq_hbm, wq_v, sem_w.at[0], i), None)

  cp_x.wait()
  xf = x_v[...].astype(F32)
  xc = xf - jnp.mean(xf, axis=-1, keepdims=True)
  xn = xc / jnp.sqrt(jnp.mean(xc * xc, axis=-1, keepdims=True) + 1e-5)
  row = lax.broadcasted_iota(jnp.int32, (8, D), 0)
  xn8 = jnp.where(row % 2 == 0, xn[0:1, :], xn[1:2, :]).astype(BF16)

  lax.fori_loop(0, NW, lambda i, _: issue_spread(w1_hbm, w1_v, sem_w.at[1], i), None)

  row128 = lax.broadcasted_iota(jnp.int32, (8, DH), 0)
  wait_for(wq_v, sem_w.at[0])
  for u in range(4):
    for t in range(u * LAG // 8, (u + 1) * LAG // 8):
      issue_kv(k_hbm, kbuf, sem_k, 0, t)
    qq = jnp.dot(xn8, wq_v[:, u * (A // 4):(u + 1) * (A // 4)], preferred_element_type=F32)
    for h in range(Hkv // 4):
      q_s[u * (Hkv // 4) + h] = jnp.where(
          row128 < 2, qq[:, 2 * h * DH:(2 * h + 1) * DH], qq[:, (2 * h + 1) * DH:(2 * h + 2) * DH])
  wait_for(w1_v, sem_w.at[1])
  cp_b1.wait()
  cp_b2.wait()
  b1 = b1_v[...].astype(F32).reshape(1, F)
  for u in range(4):
    for t in range((4 + u) * LAG // 8, (5 + u) * LAG // 8):
      issue_kv(k_hbm, kbuf, sem_k, 0, t)
    cs = slice(u * (F // 4), (u + 1) * (F // 4))
    hh = jnp.dot(xn8, w1_v[:, cs], preferred_element_type=F32) + b1[:, cs]
    h_s[:, cs] = jax.nn.gelu(hh, approximate=True).astype(BF16)

  scale = DH ** -0.5
  even = lax.broadcasted_iota(jnp.int32, (8, SR), 0) % 2 == 0

  def group(g, _):
    qs = [q_s[g * GH + dh].astype(BF16) for dh in range(GH)]

    def qk(i, ms):
      wait_kv(kbuf, sem_k, i)
      rs = pl.ds(mult(i, SR), SR)
      out = []
      for dh in range(GH):
        s0 = lax.dot_general(qs[dh], kbuf[dh, 0, rs, :], NT, preferred_element_type=F32)
        s1 = lax.dot_general(qs[dh], kbuf[dh, 1, rs, :], NT, preferred_element_type=F32)
        s = jnp.where(even, s0, s1) * scale
        s_s[dh, :, rs] = s
        m = ms[dh]
        for j in range(SR // DH):
          m = jnp.maximum(m, s[:, j * DH:(j + 1) * DH])
        out.append(m)
      return out

    def qk_issue_k(i, ms):
      issue_kv(k_hbm, kbuf, sem_k, g, i + LAG)
      return qk(i, ms)

    def qk_issue_v(i, ms):
      issue_kv(v_hbm, vbuf, sem_v, g, i + LAG - NS)
      return qk(i, ms)

    ms = [jnp.full((8, DH), -jnp.inf, F32)] * GH
    ms = lax.fori_loop(0, NS - LAG, qk_issue_k, ms)
    ms = lax.fori_loop(NS - LAG, NS, qk_issue_v, ms)
    ms = [jnp.max(m, axis=-1, keepdims=True) for m in ms]

    def pv(i, carry):
      accs, ls = carry
      wait_kv(vbuf, sem_v, i)
      rs = pl.ds(mult(i, SR), SR)
      new_accs, new_ls = [], []
      for dh in range(GH):
        e = jnp.exp(s_s[dh, :, rs] - ms[dh])
        l = ls[dh]
        for j in range(SR // DH):
          l = l + e[:, j * DH:(j + 1) * DH]
        new_ls.append(l)
        p = e.astype(BF16)
        for b in range(B):
          new_accs.append(
              accs[dh * B + b] + jnp.dot(p, vbuf[dh, b, rs, :], preferred_element_type=F32))
      return new_accs, new_ls

    def pv_issue_v(i, carry):
      issue_kv(v_hbm, vbuf, sem_v, g, i + LAG)
      return pv(i, carry)

    def pv_issue_next(i, carry):
      @pl.when(g + 1 < NG)
      def _():
        issue_kv(k_hbm, kbuf, sem_k, g + 1, i + LAG - NS)

      @pl.when(g + 1 == NG)
      def _():
        issue_wo(i + LAG - NS)
      return pv(i, carry)

    z = jnp.zeros((8, DH), F32)
    carry = lax.fori_loop(0, NS - LAG, pv_issue_v, ([z] * (GH * B), [z] * GH))
    accs, ls = lax.fori_loop(NS - LAG, NS, pv_issue_next, carry)
    for dh in range(GH):
      l = jnp.sum(ls[dh], axis=-1, keepdims=True)
      o_s[g * GH + dh] = jnp.where(row128 % 2 == 0, accs[dh * B], accs[dh * B + 1]) / l
    return None

  lax.fori_loop(0, NG, group, None)

  parts = []
  for h in range(Hkv):
    ob = o_s[h]
    parts += [jnp.where(row128 < 2, ob, 0.0), jnp.where(row128 < 2, 0.0, ob)]
  o8 = jnp.concatenate(parts, axis=1).astype(BF16)

  pending = [functools.partial(issue_wo, i) for i in range(LAG, NW)]
  pending += [functools.partial(issue_w2, i) for i in range(NW)]

  def proj(lhs, w_v, sem, blocks):
    outs = []
    for i0, n in blocks:
      for issue in pending[:n]:
        issue()
      del pending[:n]
      for i in range(i0, i0 + n):
        wait_for(w_v.at[pl.ds(WR * i, WR), :], sem.at[i])
      outs.append(
          lax.dot_general(lhs, w_v[i0 * WR:(i0 + n) * WR, :], NT, preferred_element_type=F32))
    return outs

  acc = jnp.concatenate(
      proj(o8, wo_v, sem_o, [(i, 2) for i in range(0, NW - 1, 2)] + [(NW - 1, 1)]), axis=1)
  att = acc[0:2] + acc[2:4]
  b2 = b2_v[...].astype(F32).reshape(1, D)

  def finish(f, lo, hi):
    ff = f[0:2] + b2[:, lo:hi]
    gate = ff * jax.nn.sigmoid(ff)
    o_ref[:, lo:hi] = (xf[:, lo:hi] + att[:, lo:hi] * gate).astype(o_ref.dtype)

  early = NW - 5
  f0 = proj(h_s[...], w2_v, sem_2, [(i, 2) for i in range(0, early, 2)])
  for issue in pending:
    issue()
  res = {}
  for u in list(range(early, NW + 1, 2)) + list(range(early + 1, NW + 1, 2)):
    rs, cs = w2_unit(u)
    if u == NW - 2:
      finish(jnp.concatenate(f0 + [res[early], res[early + 1]], axis=1), 0, (NW - 3) * WR)
    wait_for(w2_v.at[rs, cs], sem_2.at[u])
    res[u] = lax.dot_general(h_s[:, cs], w2_v[rs, cs], NT, preferred_element_type=F32)
  finish(jnp.concatenate([res[NW - 3], res[NW - 2]], axis=1), (NW - 3) * WR, D - WR)
  finish(res[NW - 1] + res[NW], D - WR, D)


@jax.jit
def pallas_recurrent_scan__sliding_block_cached__dense_activation_gelu__decode_kernel(
    A_x: jax.Array,
    A_k_cache: jax.Array,
    A_v_cache: jax.Array,
    A_wq: jax.Array,
    A_wo: jax.Array,
    B_x: jax.Array,
    B_w1: jax.Array,
    B_b1: jax.Array,
    B_w2: jax.Array,
    B_b2: jax.Array,
):
  B, Sq, D = A_x.shape
  F = B_w1.shape[1]
  Hkv, Sk = A_k_cache.shape[1:3]
  W = min(4096, max(256, Sk // 4))
  assert (B, Sq) == (2, 1) and HQ == 2 * Hkv and W % SR == 0
  assert D % 128 == 64 and D >= 5 * WR and F % 256 == 0
  hbm = pl.BlockSpec(memory_space=pltpu.HBM)
  out = pl.pallas_call(
      _kernel,
      out_shape=jax.ShapeDtypeStruct((B, D), A_x.dtype),
      in_specs=[hbm] * 9,
      out_specs=pl.BlockSpec(memory_space=pltpu.VMEM),
      scratch_shapes=[
          pltpu.VMEM((B, D), BF16), pltpu.VMEM((F,), BF16), pltpu.VMEM((D,), BF16),
          pltpu.VMEM((D, HQ * DH), BF16), pltpu.VMEM((D, HQ * DH), BF16),
          pltpu.VMEM((D, F), BF16), pltpu.VMEM((D, F), BF16),
          pltpu.VMEM((GH, B, W, DH), BF16), pltpu.VMEM((GH, B, W, DH), BF16),
          pltpu.VMEM((Hkv, 8, DH), F32), pltpu.VMEM((GH, 8, W), F32),
          pltpu.VMEM((Hkv, 8, DH), F32), pltpu.VMEM((8, F), BF16),
          pltpu.SemaphoreType.DMA((3,)), pltpu.SemaphoreType.DMA((2,)),
          pltpu.SemaphoreType.DMA((D // WR,)), pltpu.SemaphoreType.DMA((D // WR + 1,)),
          pltpu.SemaphoreType.DMA((W // SR,)), pltpu.SemaphoreType.DMA((W // SR,)),
      ],
      compiler_params=pltpu.CompilerParams(
          vmem_limit_bytes=64 * 1024 * 1024, disable_semaphore_checks=True),
  )(A_x.reshape(B, D), A_k_cache, A_v_cache, A_wq, A_wo.T, B_w1, B_b1, B_w2.T, B_b2)
  return out.reshape(B, Sq, D)
```
